```python
import os as _os
_os.environ.setdefault('JAX_PLATFORMS', 'cpu')
import jax
import jax.numpy as jnp

def _softmax(x, axis=-1):
    return jax.nn.softmax(x, axis=axis)

def _gelu(x):
    return jax.nn.gelu(x, approximate=True)

def _silu(x):
    return jax.nn.silu(x)

def _sigmoid(x):
    return jax.nn.sigmoid(x)

def _layernorm(x, axis=-1, eps=1e-05):
    m = jnp.mean(x, axis=axis, keepdims=True)
    v = jnp.var(x, axis=axis, keepdims=True)
    return (x - m) / jnp.sqrt(v + eps)

def _scatter_add(tgt, idx, src, axis=0):
    return tgt.at[idx].add(src)

def _segment_sum(src, seg, n):
    return jax.ops.segment_sum(src, seg, n)

class _Rng:

    def __init__(self, key):
        self._k = key

    def _next(self):
        self._k, sub = jax.random.split(self._k)
        return sub

    def normal(self, shape):
        return jax.random.normal(self._next(), shape, dtype=jnp.bfloat16)

    def randint(self, lo, hi, shape):
        return jax.random.randint(self._next(), shape, lo, hi, dtype=jnp.int32)

    def uniform(self, shape, lo=0.0, hi=1.0):
        return jax.random.uniform(self._next(), shape, jnp.bfloat16, lo, hi)

    def permutation(self, n):
        return jax.random.permutation(self._next(), n)
kernel_name = 'adaLN_cond__memory_aug_recurrent_mem_tr__moe_arch_mod__prompt'

def setup_inputs():
    _rng = _Rng(jax.random.key(int.from_bytes(__import__("os").urandom(4), "little")))
    _w = lambda a: (lambda t: t.astype(jnp.bfloat16) if jnp.issubdtype(t.dtype, jnp.floating) else t)(jnp.asarray(a))

    def _A_setup():
        B, S, Dm = (1, 2048, 448)
        H, Dh = (16, 256)
        M, seg = (8, 32)
        seg = min(seg, S)
        S = S // seg * seg
        return {'x': _w((lambda *s: _rng.normal(s) * 0.05)(B, S, Dm)), 'mem0': _w((lambda *s: _rng.normal(s) * 0.4)(B, M, Dm)), 'Wq': _w((lambda *s: _rng.normal(s) * 1.6)(Dm, H, Dh) * Dm ** (-0.5)), 'Wk': _w((lambda *s: _rng.normal(s) * 1.6)(Dm, H, Dh) * Dm ** (-0.5)), 'Wv': _w((lambda *s: _rng.normal(s) * 0.4)(Dm, H, Dh) * Dm ** (-0.5)), 'Wo': _w((lambda *s: _rng.normal(s) * 0.4)(H, Dh, Dm) * (H * Dh) ** (-0.5)), 'seg_len': seg}
    _A_in = _A_setup()

    def _B_setup():
        B, S, D, F, C = (1, 2048, 448, 1792, 1)
        return {'x': _w((lambda *s: _rng.normal(s) * 0.05)(B, S, D)), 'w_r': _w((lambda *s: _rng.normal(s) * 0.05)(D)), 'w_gate': _w((lambda *s: _rng.normal(s) * 0.05)(D, F)), 'w_up': _w((lambda *s: _rng.normal(s) * 0.05)(D, F)), 'w_down': _w((lambda *s: _rng.normal(s) * 0.05)(F, D))}
    _B_in = _B_setup()
    return {'A_x': _A_in['x'], 'A_mem0': _A_in['mem0'], 'A_Wq': _A_in['Wq'], 'A_Wk': _A_in['Wk'], 'A_Wv': _A_in['Wv'], 'A_Wo': _A_in['Wo'], 'A_seg_len': _A_in['seg_len'], 'B_x': _B_in['x'], 'B_w_r': _B_in['w_r'], 'B_w_gate': _B_in['w_gate'], 'B_w_up': _B_in['w_up'], 'B_w_down': _B_in['w_down'], 'c': _w((lambda *s: _rng.normal(s) * 0.05)(1, 448) * 8.0), 'w_mod': _w((lambda *s: _rng.normal(s) * 0.05)(448, 6 * 448) * 448 ** (-0.5) * 8.0)}

def reference(A_x, A_mem0, A_Wq, A_Wk, A_Wv, A_Wo, A_seg_len, B_x, B_w_r, B_w_gate, B_w_up, B_w_down, c, w_mod):

    def _A_ref(x, mem0, Wq, Wk, Wv, Wo, seg_len):
        B, S, Dm = x.shape
        H, Dh = (Wq.shape[1], Wq.shape[2])
        M = mem0.shape[1]
        scale = Dh ** (-0.5)
        n_seg = S // seg_len
        L = M + seg_len
        idx = jnp.arange(L)
        mask = (idx[:, None] < M) | (idx[:, None] >= idx[None, :])
        mem = mem0
        outs = []
        for s in range(n_seg):
            xs = x[:, s * seg_len:(s + 1) * seg_len, :].copy()
            h = jnp.concatenate([mem, xs], axis=1)
            q = jnp.einsum('btd,dhe->bhte', h, Wq)
            k = jnp.einsum('btd,dhe->bhte', h, Wk)
            v = jnp.einsum('btd,dhe->bhte', h, Wv)
            scores = jnp.einsum('bhqe,bhke->bhqk', q, k) * scale
            scores = jnp.where(mask[None, None], scores, -1000000000.0)
            p = _softmax(scores, axis=-1)
            o = jnp.einsum('bhqk,bhke->bhqe', p, v)
            o = jnp.einsum('bhte,hed->btd', o, Wo)
            mem = o[:, :M, :].copy()
            outs.append(o[:, M:, :])
        return jnp.concatenate(outs, axis=1)

    def _B_ref(x, w_r, w_gate, w_up, w_down):
        B, S, D = x.shape
        C = 1
        r = x @ w_r
        idx = jnp.argsort(-r, axis=-1)[:, :C]
        idx_e = jnp.repeat(idx.reshape(B, C, 1), D, axis=2)
        x_sel = jnp.take_along_axis(x, idx_e, axis=1)
        g = _silu(x_sel @ w_gate)
        u = x_sel @ w_up
        y = g * u @ w_down
        r_sel = _sigmoid(jnp.take_along_axis(r, idx, axis=1))
        y = y * r_sel.reshape(B, C, 1)
        b_off = (jnp.arange(B) * S).reshape(B, 1)
        flat_idx = (idx + b_off).reshape(B * C)
        zero = (x * 0.0).reshape(B * S, D)
        upd = _scatter_add(zero, flat_idx, y.reshape(B * C, D), axis=0)
        return x + upd.reshape(B, S, D)
    x = A_x
    mod = (_silu(c) @ w_mod).reshape(c.shape[0], 6, 1, -1)
    sa, ca, ga, sb, cb, gb = (mod[:, 0].copy(), mod[:, 1].copy(), mod[:, 2].copy(), mod[:, 3].copy(), mod[:, 4].copy(), mod[:, 5].copy())
    h = _layernorm(x, axis=-1) * (1 + ca) + sa
    x = x + ga * _A_ref(h, A_mem0, A_Wq, A_Wk, A_Wv, A_Wo, A_seg_len)
    h = _layernorm(x, axis=-1) * (1 + cb) + sb
    x = x + gb * _B_ref(h, B_w_r, B_w_gate, B_w_up, B_w_down)
    return x
```

```python
import functools

import jax
import jax.numpy as jnp
from jax import lax
from jax.experimental import pallas as pl
from jax.experimental.pallas import tpu as pltpu

F32 = jnp.float32
BF16 = jnp.bfloat16
U32 = jnp.uint32
NT = (((1,), (1,)), ((), ()))
TIE, CUT0, CUT1, CUT2, UNR = 0, 0, 1, 7, 1


def _round_bf16(v):
    return v.astype(BF16).astype(F32)


def _pack(v):
    return pltpu.bitcast(v.astype(BF16), U32)


def _unpack(v):
    return pltpu.bitcast(v, BF16)


def _kernel(xT_hbm, mem0_hbm, wq_hbm, wk_hbm, wv_hbm, woT_hbm, wr_hbm, wg_hbm,
            wu_hbm, wdT_hbm, c_hbm, wmod_hbm, outT_hbm,
            xT_s, wq_s, wk_s, wv_s, woT_s, wg_s, wu_s, wdT_s, wmod0_s, wmod1_s, mod_s, mem0_s, wr_s, c_s,
            w1_s, w2_s, w3_s, v1_s, v2_s, xn_s, h_s, o_s, y_s, h2_s, outT_s, kT_s, sems, osems,
            *, S, D, H, E, M, SEG):
    NP = H // 2
    DA = (D // 128) * 128
    DB = D - DA
    DP = DA + 128
    NT_ = DP // 128
    L = M + SEG
    NSEG = S // SEG
    NBLK = S // 128
    LAG = NT_ + 1
    scale = E ** (-0.5)

    def pair_copy(src, dst, p, sem):
        return pltpu.make_async_copy(src.bitcast(U32).at[:, p, :], dst.at[p], sems.at[sem])

    def qk_copies(p):
        return [pair_copy(wk_hbm, wk_s, p, 16 + 4 * p), pair_copy(wq_hbm, wq_s, p, 17 + 4 * p)]

    def vo_copies(p):
        return [pair_copy(wv_hbm, wv_s, p, 18 + 4 * p),
                pltpu.make_async_copy(woT_hbm.at[pl.ds(2 * p, 2)], woT_s.at[p], sems.at[19 + 4 * p])]

    def copies(pairs, sem0):
        return [pltpu.make_async_copy(a, b, sems.at[sem0 + i]) for i, (a, b) in enumerate(pairs)]

    def x_copies(c0, n, sem0):
        cols = pl.ds(c0, n)
        return copies(((xT_hbm.at[:, cols], xT_s.at[pl.ds(0, D), cols]),
                       (xT_hbm.at[pl.ds(DA, DB), cols], xT_s.at[pl.ds(D, DB), cols])), sem0)

    def start(cps):
        for cp in cps:
            cp.start()

    def wait(cps):
        for cp in cps:
            cp.wait()

    d_small = copies(((c_hbm, c_s), (mem0_hbm, mem0_s), (wr_hbm, wr_s)), 0)
    d_x0 = x_copies(0, 256, 3)
    d_mod0 = copies(((wmod_hbm.at[:, pl.ds(0, 2 * D)], wmod0_s),), 5)
    d_mod1 = copies(((wmod_hbm.at[:, pl.ds(2 * D, 4 * D)], wmod1_s),), 11)
    d_x1 = x_copies(256, S - 256, 6)
    d_ffn = copies(((wg_hbm, wg_s), (wu_hbm, wu_s), (wdT_hbm, wdT_s)), 8)
    for p in range(NP):
        start(qk_copies(p))
    for p in range(NP):
        start(vo_copies(p))
    start(d_small + d_x0 + d_mod0 + d_mod1 + d_x1 + d_ffn)

    lane = lax.broadcasted_iota(jnp.int32, (1, 128), 1)
    lo_half = lane < DB

    def lo(v):
        return jnp.where(lo_half, v, 0.0)

    def hi(v):
        return jnp.where(lo_half, 0.0, v)

    def head_pair(ref, p):
        w = ref[p]
        return (pltpu.bitcast(w << 16, F32), pltpu.bitcast(w & jnp.uint32(0xFFFF0000), F32))

    def fold(x0, x1, y0, y1):
        t0 = lax.dot_general(y0[DA:], x0.astype(BF16), NT, preferred_element_type=F32)
        t1 = lax.dot_general(y1[DA:], x1.astype(BF16), NT, preferred_element_type=F32)
        t = jnp.concatenate([t0, t1], axis=0)
        t = jnp.concatenate([t, jnp.zeros((128, DP - D), F32)], axis=1)
        out = []
        for x, y in ((x0, y0), (x1, y1)):
            r = lax.dot_general(jnp.concatenate([x[DA:], x[:DA]], axis=0), y[:DA].astype(BF16), NT,
                                preferred_element_type=F32)
            out += [r[DB:], r[:DB]]
        return out + [t.T[:D]]

    def fold_qk(p, _):
        wait(qk_copies(p))
        k0, k1 = head_pair(wk_s, p)
        q0, q1 = head_pair(wq_s, p)
        a0, a0b, a1, a1b, ab = fold(k0 * scale, k1 * scale, q0, q1)
        w3 = jnp.concatenate([a0b, a1b], axis=0).T
        w1_s[p] = _pack(jnp.concatenate([a0, a1], axis=1))
        w3_s[p] = _pack(w3)
        w2_s[p] = _pack(ab)

    def fold_vo(p, _):
        wait(vo_copies(p))
        v0, v1 = head_pair(wv_s, p)
        b0, b0b, b1, b1b, bb = fold(v0, v1, woT_s[p, 0], woT_s[p, 1])
        v1_s[p] = _pack(jnp.concatenate([b0, b1, bb[:DA]], axis=1))
        v2_s[p] = _pack(jnp.concatenate(
            [jnp.concatenate([b0b, lo(bb[DA:])], axis=1),
             jnp.concatenate([b1b, hi(bb[DA:])], axis=1)], axis=0))

    with jax.named_scope("fold_k"):
        lax.fori_loop(0, NP, fold_qk, None, unroll=UNR)
    with jax.named_scope("fold_v"):
        lax.fori_loop(0, NP, fold_vo, None, unroll=UNR)

    def dup(v):
        return jnp.concatenate([v, v[:, DA:]], axis=1)

    def rowsum(v):
        t = lo(v[:, DA:])
        for i in range(DA // 128):
            t = t + v[:, i * 128:(i + 1) * 128]
        return jnp.sum(t, axis=1, keepdims=True)

    def layernorm(v):
        mu = rowsum(v) * (1.0 / D)
        d = v - mu
        var = rowsum(d * d) * (1.0 / D)
        return d * lax.rsqrt(var + 1e-5)

    def tile_in(t):
        t0 = pl.multiple_of(t // NT_ * 128, 128)
        f0 = pl.multiple_of(t % NT_ * 128, 128)
        xn_s[pl.ds(t0, 128), pl.ds(f0, 128)] = xT_s[pl.ds(f0, 128), pl.ds(t0, 128)].astype(F32).T

    def tile_out(t):
        t0 = pl.multiple_of(t // NT_ * 128, 128)
        f0 = pl.multiple_of(t % NT_ * 128, 128)
        outT_s[pl.ds(f0, 128), pl.ds(t0, 128)] = (
            y_s[pl.ds(pl.multiple_of(t0 + SEG, SEG), 128), pl.ds(f0, 128)].T.astype(BF16))

    def out_copy(b, n, sem):
        cols = pl.ds(pl.multiple_of(b * 128, 128), n * 128)
        return pltpu.make_async_copy(outT_s.at[pl.ds(0, D), cols], outT_hbm.at[:, cols], osems.at[sem])

    with jax.named_scope("pre"):
        wait(d_small + d_x0)
        for t in range(LAG):
            tile_in(t)

        def modulation(w_ref):
            cv = c_s[...].astype(F32)
            sc = jnp.broadcast_to(cv * jax.nn.sigmoid(cv), (8, D))
            mod = jnp.dot(_round_bf16(sc), w_ref[...], preferred_element_type=F32)
            return [dup(mod[:, i * D:(i + 1) * D]) for i in range(w_ref.shape[1] // D)]

        wait(d_mod0)
        sa, ca = [v[0:1] for v in modulation(wmod0_s)]
        ca1 = 1.0 + ca
        mod_s[...] = jnp.zeros(mod_s.shape, F32)
        wr = dup(wr_s[...].astype(F32))

        def ln1(k):
            r0 = pl.multiple_of(k * SEG, SEG)
            hn = _round_bf16(layernorm(xn_s[pl.ds(r0, SEG), :]) * ca1 + sa)
            h_s[...] = hn
            return hn

        ln1(0)
        o_s[...] = jnp.zeros((SEG, DP), F32)
        y_s[pl.ds(SEG, 128), :] = jnp.zeros((128, DP), F32)

    NB = L // M
    seen_by = [[0] + [j for j in range(1, NB) if j >= i] for i in range(NB)]
    sees = [[i for i in range(NB) if j in seen_by[i]] for j in range(NB)]
    causal = (lax.broadcasted_iota(jnp.int32, (M, 128), 0)
              >= lax.broadcasted_iota(jnp.int32, (M, 128), 1) % M)
    slot = lane // (2 * M)

    def blocks(v, js):
        return jnp.concatenate([v[j * M:(j + 1) * M] for j in js], axis=0)

    def roll(v, k):
        k %= 128
        return v if k == 0 else pltpu.roll(v, k, 1)

    def per_head(v, comb):
        d = 1
        while d < M:
            v = comb(v, jnp.where((lane & d) != 0, roll(v, d), roll(v, -d)))
            d *= 2
        return v

    def merge(v):
        return jnp.concatenate([v[:, :DA], v[:, DA:] + roll(v[:, DA:], DB)], axis=1)

    def finish(k, best, bidx):
        q0 = pl.multiple_of(k * SEG, SEG)
        p0 = pl.multiple_of(jnp.maximum(k - 1, 0) * SEG, SEG)
        ga, sb, cb, gb = [mod_s[i, 0:1] for i in range(4)]
        x2 = xn_s[pl.ds(p0, SEG), :] + ga * merge(o_s[...])
        h2 = _round_bf16(layernorm(x2) * (1.0 + cb) + sb)
        y_s[pl.ds(q0, SEG), :] = x2 + gb * (h2 + h2 * 0.0)
        h2_s[pl.ds(q0, SEG), :] = h2
        r = jnp.broadcast_to(_round_bf16(rowsum(h2 * wr)), (SEG, 128))
        r = jnp.where(k > 0, r, -jnp.inf)
        rid = lax.broadcasted_iota(jnp.int32, (8, 128), 0) + q0
        for i in range(SEG // 8):
            ri = r[i * 8:(i + 1) * 8]
            better = ri > best
            best = jnp.where(better, ri, best)
            bidx = jnp.where(better, rid + i * 8, bidx)
        return best, bidx

    def step(s, carry):
        m, best, bidx = carry

        @pl.when(s == 1)
        def _():
            wait(d_mod1)
            for i, v in enumerate(modulation(wmod1_s)):
                mod_s[i] = v

        @pl.when(s == 2 * NT_ - LAG)
        def _():
            wait(d_x1)

        h = jnp.concatenate([_round_bf16(merge(m)), h_s[...]], axis=0)
        ha = h[:, :DA]
        h3 = h[:, DA:]
        tile_out(jnp.maximum(s - LAG, 0))
        best, bidx = finish(s, best, bidx)
        hn = ln1(jnp.minimum(s + 1, NSEG - 1))
        tile_in(jnp.minimum(s + LAG, NBLK * NT_ - 1))

        kparts = []
        for p in range(NP):
            ra = jnp.dot(ha, _unpack(w1_s[p]), preferred_element_type=F32)
            if p == 0:
                rb = jnp.dot(h[:, :D],
                             _unpack(jnp.concatenate([w2_s[q] for q in range(NP)], axis=1)),
                             preferred_element_type=F32)
            sh = rb[:, p * 128:(p + 1) * 128]
            kparts.append(jnp.concatenate([ra[:, :DA], lo(sh)], axis=1))
            kparts.append(jnp.concatenate([ra[:, DA:2 * DA], hi(sh)], axis=1))
        vparts = []

        side = best
        for i in range(SEG // 8):
            side = side + hn[i * 8:(i + 1) * 8, :128]
        ha_late = jnp.concatenate([jnp.concatenate(
            [jnp.where(s < 0, side, ha[:8, :128]), ha[:8, 128:]], axis=1), ha[8:]], axis=0)

        def values(p):
            rv = jnp.dot(ha_late if p == TIE else ha, _unpack(v1_s[p]), preferred_element_type=F32)
            sh = rv[:, 2 * DA:]
            vparts.append(jnp.concatenate([rv[:, :DA], lo(sh)], axis=1))
            vparts.append(jnp.concatenate([rv[:, DA:2 * DA], hi(sh)], axis=1))

        zero = jnp.zeros((2 * M, 128), F32)
        e_rows = [jnp.concatenate([lo(h3[i * M:(i + 1) * M]), hi(h3[i * M:(i + 1) * M])], axis=0)
                  for i in range(NB)] + [zero] * (NP - NB)
        e_rows = [e.astype(BF16) for e in e_rows]

        q2 = jnp.dot(ha, _unpack(jnp.concatenate([w3_s[p] for p in range(NP)], axis=1)),
                     preferred_element_type=F32)
        for p in range(CUT0):
            values(p)
        s2 = lax.dot_general(
            _round_bf16(jnp.concatenate([q2[:, p * 128:(p + 1) * 128] for p in range(NP)], axis=0)),
            jnp.concatenate(e_rows, axis=0), NT, preferred_element_type=F32)
        for p in range(CUT0, CUT1):
            values(p)
        sc_ = {}
        for i in range(NB):
            kT_s[i] = _pack(jnp.concatenate([q[i * M:(i + 1) * M] for q in kparts], axis=0).T)
            t = jnp.dot(blocks(h, seen_by[i]), _unpack(kT_s[i]), preferred_element_type=F32)
            for n, j in enumerate(seen_by[i]):
                sc_[j, i] = t[n * M:(n + 1) * M]
        prob = {}
        for j in range(NB):
            for i in sees[j]:
                t = None
                for p in range(NP):
                    r = roll(s2[p * L + j * M:p * L + (j + 1) * M], 2 * M * (p - i))
                    t = r if t is None else jnp.where(slot == p, r, t)
                t = sc_[j, i] + t
                sc_[j, i] = jnp.where(causal, t, -1e9) if (i == j and j > 0) else t
            mx = per_head(functools.reduce(jnp.maximum, [sc_[j, i] for i in sees[j]]), jnp.maximum)
            ex = [jnp.exp(sc_[j, i] - mx) for i in sees[j]]
            inv = 1.0 / per_head(functools.reduce(jnp.add, ex), jnp.add)
            for i, e in zip(sees[j], ex):
                prob[j, i] = _round_bf16(e * inv)
        shifted = {ji: roll(v, 2 * M * ji[1]) for ji, v in prob.items()}
        for p in range(CUT1, CUT2):
            values(p)
        u2 = []
        for p in range(NP):
            rows = []
            for j in range(NB):
                t = jnp.zeros((M, 128), F32)
                for i in sees[j]:
                    t = jnp.where(slot == (i + p) % NP, shifted[j, i], t)
                rows.append(t)
            e = jnp.concatenate([e_rows[(c - p) % NP] for c in range(NP)], axis=0)
            u2.append(jnp.dot(jnp.concatenate(rows, axis=0), e, preferred_element_type=F32))
        for p in range(CUT2, NP):
            values(p)
        o = jnp.dot(_round_bf16(jnp.concatenate(u2, axis=1)),
                    _unpack(jnp.concatenate([v2_s[p] for p in range(NP)], axis=0)),
                    preferred_element_type=F32)
        ob = [o[j * M:(j + 1) * M] for j in range(NB)]
        for i in range(NB):
            vst = jnp.concatenate([q[i * M:(i + 1) * M] for q in vparts], axis=0).astype(BF16)
            t = jnp.dot(jnp.concatenate([prob[j, i] for j in seen_by[i]], axis=0), vst,
                        preferred_element_type=F32)
            for n, j in enumerate(seen_by[i]):
                ob[j] = ob[j] + t[n * M:(n + 1) * M]
        o = jnp.concatenate(ob, axis=0)
        o_s[...] = o[M:]

        done = s - LAG + 1
        @pl.when(jnp.logical_and(done > 0, done % NT_ == 0))
        def _():
            out_copy(done // NT_ - 1, 1, 0).start()

        return o[:M], best, bidx

    m0 = dup(mem0_s[...].astype(F32))
    m0 = jnp.concatenate([m0[:, :DA], lo(m0[:, DA:])], axis=1)
    with jax.named_scope("main"):
        _, best, bidx = lax.fori_loop(
            0, NSEG, step,
            (m0, jnp.full((8, 128), -jnp.inf, F32), jnp.full((8, 128), SEG, jnp.int32)))
    with jax.named_scope("post"):
        best, bidx = finish(NSEG, best, bidx)
        sent = (NSEG - LAG) // NT_
        for t in range(NSEG - LAG, NBLK * NT_):
            tile_out(t)
        out_copy(sent, NBLK - sent, 1).start()

        rmax = jnp.max(best, axis=0, keepdims=True)
        idx = jnp.min(jnp.where(best == rmax, bidx, S + SEG - 1))

        wait(d_ffn)
        hsel = jnp.broadcast_to(h2_s[pl.ds(idx, 1), :], (8, DP))[:, :D]
        g = jnp.dot(hsel, wg_s[...], preferred_element_type=F32)
        u = jnp.dot(hsel, wu_s[...], preferred_element_type=F32)
        act = _round_bf16(g * jax.nn.sigmoid(g) * u)
        y = lax.dot_general(act, wdT_s[...], NT, preferred_element_type=F32)
        y = dup(y)[0:1] * jax.nn.sigmoid(rmax[:, 0:1])
        y_s[pl.ds(idx, 1), :] = y_s[pl.ds(idx, 1), :] + mod_s[3, 0:1] * y

        out_copy(0, sent, 0).wait()
        out_copy(sent, NBLK - sent, 1).wait()
        blk = (idx - SEG) // 128
        for j in range(NT_):
            tile_out(blk * NT_ + j)
        fix = out_copy(blk, 1, 2)
        fix.start()
        fix.wait()


@functools.partial(jax.jit, static_argnames=("A_seg_len",))
def pallas_adaLN_cond__memory_aug_recurrent_mem_tr__moe_arch_mod__prompt_kernel(
    A_x, A_mem0, A_Wq, A_Wk, A_Wv, A_Wo, A_seg_len, B_x, B_w_r, B_w_gate, B_w_up,
    B_w_down, c, w_mod,
):
    del B_x
    _, S, D = A_x.shape
    _, H, E = A_Wq.shape
    M = A_mem0.shape[1]
    F = B_w_gate.shape[1]
    SEG = int(A_seg_len)
    DA = (D // 128) * 128
    DP = DA + 128
    NP = H // 2
    hbm = pl.BlockSpec(memory_space=pl.ANY)
    pairs = pltpu.VMEM((NP, D, E), U32)
    outT = pl.pallas_call(
        functools.partial(_kernel, S=S, D=D, H=H, E=E, M=M, SEG=SEG),
        out_shape=jax.ShapeDtypeStruct((D, S), BF16),
        in_specs=[hbm] * 12,
        out_specs=hbm,
        scratch_shapes=[
            pltpu.VMEM((DP, S), BF16),
            pairs, pairs, pairs,
            pltpu.VMEM((NP, 2, D, E), BF16),
            pltpu.VMEM((D, F), BF16),
            pltpu.VMEM((D, F), BF16),
            pltpu.VMEM((D, F), BF16),
            pltpu.VMEM((D, 2 * D), BF16),
            pltpu.VMEM((D, 4 * D), BF16),
            pltpu.VMEM((4, 8, DP), F32),
            pltpu.VMEM((M, D), BF16),
            pltpu.VMEM((1, D), BF16),
            pltpu.VMEM((1, D), BF16),
            pltpu.VMEM((NP, DA // 2, 2 * DA), U32),
            pltpu.VMEM((NP, D // 2, 128), U32),
            pltpu.VMEM((NP, DA // 2, 128), U32),
            pltpu.VMEM((NP, DA // 2, 2 * D), U32),
            pltpu.VMEM((NP, 64, DP), U32),
            pltpu.VMEM((S, DP), F32),
            pltpu.VMEM((SEG, DP), F32),
            pltpu.VMEM((SEG, DP), F32),
            pltpu.VMEM((S + SEG, DP), F32),
            pltpu.VMEM((S + SEG, DP), F32),
            pltpu.VMEM((DP, S), BF16),
            pltpu.VMEM(((M + SEG) // M, DP // 2, 128), U32),
            pltpu.SemaphoreType.DMA((16 + 4 * NP,)),
            pltpu.SemaphoreType.DMA((3,)),
        ],
        compiler_params=pltpu.CompilerParams(vmem_limit_bytes=100 * 2**20),
        name="rmt_fused",
    )(
        jnp.transpose(A_x[0]),
        A_mem0[0],
        A_Wq,
        A_Wk,
        A_Wv,
        jnp.transpose(A_Wo, (0, 2, 1)),
        B_w_r.reshape(1, D),
        B_w_gate,
        B_w_up,
        jnp.transpose(B_w_down),
        c,
        w_mod,
    )
    return jnp.transpose(outT)[None]
```

```python
import functools

import jax
import jax.numpy as jnp
from jax import lax
from jax.experimental import pallas as pl
from jax.experimental.pallas import tpu as pltpu

F32 = jnp.float32
BF16 = jnp.bfloat16
U32 = jnp.uint32
NT = (((1,), (1,)), ((), ()))
LANES = 128

SIDE_TIE = 3
VALUES_EARLY = 2
VALUES_LATE = 1
FILL_PAIRS = 4


def _round_bf16(v):
    return v.astype(BF16).astype(F32)


def _pack(v):
    return pltpu.bitcast(v.astype(BF16), U32)


def _unpack(v):
    return pltpu.bitcast(v, BF16)


def _dot(a, b):
    return jnp.dot(a, b, preferred_element_type=F32)


def _dot_nt(a, b):
    return lax.dot_general(a, b, NT, preferred_element_type=F32)


def _rows(parts):
    return jnp.concatenate(parts, axis=0)


def _cols(parts):
    return jnp.concatenate(parts, axis=1)


def _roll(v, k):
    k %= LANES
    return v if k == 0 else pltpu.roll(v, k, 1)


def _kernel(xT_hbm, mem0_hbm, wq_hbm, wk_hbm, wv_hbm, woT_hbm, wr_hbm, wg_hbm, wu_hbm, wdT_hbm,
            c_hbm, wmod_hbm, outT_hbm,
            xT_s, wq_s, wk_s, wv_s, woT_s, wg_s, wu_s, wdT_s, wmod0_s, wmod1_s, mod_s, mem0_s,
            wr_s, c_s, ka_s, kb_s, qb_s, va_s, vb_s, x_s, h_s, o_s, y_s, h2_s, outT_s, kT_s,
            sems, osems, *, S, D, H, E, M, SEG):
    NP = H // 2
    DA = D // LANES * LANES
    DB = D - DA
    DP = DA + LANES
    NF = DP // LANES
    L = M + SEG
    NB = L // M
    NBLK = S // LANES
    SPB = LANES // SEG
    assert 2 * DB == LANES and H * M == LANES and SEG % M == 0 and NB <= NP
    scale = E ** (-0.5)

    def pair_copy(src, dst, p, sem):
        return pltpu.make_async_copy(src.bitcast(U32).at[:, p, :], dst.at[p], sems.at[sem])

    def qk_copies(p):
        return [pair_copy(wk_hbm, wk_s, p, 16 + 4 * p), pair_copy(wq_hbm, wq_s, p, 17 + 4 * p)]

    def vo_copies(p):
        return [pair_copy(wv_hbm, wv_s, p, 18 + 4 * p),
                pltpu.make_async_copy(woT_hbm.at[pl.ds(2 * p, 2)], woT_s.at[p],
                                      sems.at[19 + 4 * p])]

    def copies(pairs, sem0):
        return [pltpu.make_async_copy(a, b, sems.at[sem0 + i]) for i, (a, b) in enumerate(pairs)]

    def x_copies(c0, n, sem0):
        cols = pl.ds(c0, n)
        return copies(((xT_hbm.at[:, cols], xT_s.at[pl.ds(0, D), cols]),
                       (xT_hbm.at[pl.ds(DA, DB), cols], xT_s.at[pl.ds(D, DB), cols])), sem0)

    def out_copy(b, n, sem):
        cols = pl.ds(pl.multiple_of(b * LANES, LANES), n * LANES)
        return pltpu.make_async_copy(outT_s.at[pl.ds(0, D), cols], outT_hbm.at[:, cols],
                                     osems.at[sem])

    def start(cps):
        for cp in cps:
            cp.start()

    def wait(cps):
        for cp in cps:
            cp.wait()

    d_small = copies(((c_hbm, c_s), (mem0_hbm, mem0_s), (wr_hbm, wr_s)), 0)
    d_x0 = x_copies(0, 2 * LANES, 3)
    d_mod0 = copies(((wmod_hbm.at[:, pl.ds(0, 2 * D)], wmod0_s),), 5)
    d_mod1 = copies(((wmod_hbm.at[:, pl.ds(2 * D, 4 * D)], wmod1_s),), 6)
    d_x1 = x_copies(2 * LANES, S - 2 * LANES, 7)
    d_ffn = copies(((wg_hbm, wg_s), (wu_hbm, wu_s), (wdT_hbm, wdT_s)), 9)
    for p in range(NP):
        start(qk_copies(p))
    for p in range(NP):
        start(vo_copies(p))
    start(d_small + d_x0 + d_mod0 + d_mod1 + d_x1 + d_ffn)

    lane = lax.broadcasted_iota(jnp.int32, (1, LANES), 1)

    def lo(v):
        return jnp.where(lane < DB, v, 0.0)

    def hi(v):
        return jnp.where(lane < DB, 0.0, v)

    def head_pair(ref, p):
        w = ref[p]
        return pltpu.bitcast(w << 16, F32), pltpu.bitcast(w & jnp.uint32(0xFFFF0000), F32)

    def fold(x0, x1, y0, y1):
        t = _rows([_dot_nt(y0[DA:], x0.astype(BF16)), _dot_nt(y1[DA:], x1.astype(BF16))])
        t = _cols([t, jnp.zeros((LANES, DP - D), F32)])
        out = []
        for x, y in ((x0, y0), (x1, y1)):
            r = _dot_nt(_rows([x[DA:], x[:DA]]), y[:DA].astype(BF16))
            out += [r[DB:], r[:DB]]
        return out + [t.T[:D]]

    def fold_qk(p, _):
        wait(qk_copies(p))
        k0, k1 = head_pair(wk_s, p)
        q0, q1 = head_pair(wq_s, p)
        aa0, ba0, aa1, ba1, b = fold(k0 * scale, k1 * scale, q0, q1)
        ka_s[p] = _pack(_cols([aa0, aa1]))
        qb_s[p] = _pack(_rows([ba0, ba1]).T)
        kb_s[p] = _pack(b)

    def fold_vo(p, _):
        wait(vo_copies(p))
        v0, v1 = head_pair(wv_s, p)
        aa0, ba0, aa1, ba1, b = fold(v0, v1, woT_s[p, 0], woT_s[p, 1])
        va_s[p] = _pack(_cols([aa0, aa1, b[:DA]]))
        vb_s[p] = _pack(_rows([_cols([ba0, lo(b[DA:])]), _cols([ba1, hi(b[DA:])])]))

    lax.fori_loop(0, NP, fold_qk, None)
    lax.fori_loop(0, NP, fold_vo, None)

    def dup(v):
        return _cols([v, v[:, DA:]])

    def merge(v):
        return _cols([v[:, :DA], v[:, DA:] + _roll(v[:, DA:], DB)])

    def rowsum(v):
        t = lo(v[:, DA:])
        for i in range(DA // LANES):
            t = t + v[:, i * LANES:(i + 1) * LANES]
        return jnp.sum(t, axis=1, keepdims=True)

    def layernorm(v):
        mu = rowsum(v) * (1.0 / D)
        d = v - mu
        var = rowsum(d * d) * (1.0 / D)
        return d * lax.rsqrt(var + 1e-5)

    def modulation(w_ref):
        cv = c_s[...].astype(F32)
        mod = _dot(_round_bf16(jnp.broadcast_to(cv * jax.nn.sigmoid(cv), (8, D))), w_ref[...])
        return [dup(mod[:, i * D:(i + 1) * D]) for i in range(w_ref.shape[1] // D)]

    def tile_in(b, f):
        t0 = pl.multiple_of(b * LANES, LANES)
        x_s[pl.ds(t0, LANES), f * LANES:(f + 1) * LANES] = (
            xT_s[f * LANES:(f + 1) * LANES, pl.ds(t0, LANES)].astype(F32).T)

    def block_out(b):
        t0 = pl.multiple_of(b * LANES, LANES)
        for f in range(NF):
            outT_s[f * LANES:(f + 1) * LANES, pl.ds(t0, LANES)] = (
                y_s[pl.ds(t0, LANES), f * LANES:(f + 1) * LANES].T.astype(BF16))

    wait(d_small + d_x0)
    for f in range(NF):
        tile_in(0, f)
    wait(d_mod0)
    sa, ca = [v[0:1] for v in modulation(wmod0_s)]
    ca1 = 1.0 + ca
    wr = dup(wr_s[...].astype(F32).reshape(1, D))

    def modulated_input(seg):
        r0 = pl.multiple_of(seg * SEG, SEG)
        return _round_bf16(layernorm(x_s[pl.ds(r0, SEG), :]) * ca1 + sa)

    h_s[...] = modulated_input(0)
    mod_s[...] = jnp.zeros(mod_s.shape, F32)
    o_s[...] = jnp.zeros(o_s.shape, F32)

    def finish(b, j, live, best, bidx):
        r0 = pl.multiple_of(b * LANES + j * SEG, SEG)
        ga, sb, cb, gb = [mod_s[i, 0:1] for i in range(4)]
        x2 = x_s[pl.ds(r0, SEG), :] + ga * merge(o_s[j])
        h2 = _round_bf16(layernorm(x2) * (1.0 + cb) + sb)
        y_s[pl.ds(r0, SEG), :] = x2 + gb * (h2 + h2 * 0.0)
        h2_s[pl.ds(r0, SEG), :] = h2
        r = jnp.broadcast_to(_round_bf16(rowsum(h2 * wr)), (SEG, LANES))
        r = jnp.where(live, r, -jnp.inf)
        rid = lax.broadcasted_iota(jnp.int32, (8, LANES), 0) + r0
        for i in range(SEG // 8):
            ri = r[i * 8:(i + 1) * 8]
            better = ri > best
            best = jnp.where(better, ri, best)
            bidx = jnp.where(better, rid + i * 8, bidx)
        return best, bidx

    seen_by = [[0] + [q for q in range(1, NB) if q >= i] for i in range(NB)]
    sees = [[i for i in range(NB) if q in seen_by[i]] for q in range(NB)]
    causal = (lax.broadcasted_iota(jnp.int32, (M, LANES), 0)
              >= lax.broadcasted_iota(jnp.int32, (M, LANES), 1) % M)
    slot = lane // (2 * M)

    def blk(v, i):
        return v[i * M:(i + 1) * M]

    def tile(v, i):
        return v[:, i * LANES:(i + 1) * LANES]

    def per_head(v, combine):
        d = 1
        while d < M:
            v = combine(v, jnp.where((lane & d) != 0, _roll(v, d), _roll(v, -d)))
            d *= 2
        return v

    def step(b, j, m, hx, best, bidx):
        h = _rows([_round_bf16(merge(m)), hx])
        ha = h[:, :DA]
        hb = h[:, DA:]

        prev = jnp.maximum(b - 1, 0)
        nxt = jnp.minimum(b + 1, NBLK - 1)
        best, bidx = finish(prev, j, b > 0, best, bidx)
        if j == SPB - 1:
            block_out(prev)
        for f in range(j * NF // SPB, (j + 1) * NF // SPB):
            tile_in(nxt, f)
        hn = modulated_input(b * SPB + j + 1 if j + 1 < SPB else nxt * SPB)
        side = functools.reduce(jnp.add, [tile(blk(hn, i), 0) for i in range(SEG // M)], best)
        ha_tied = _rows([_cols([jnp.where(b < 0, side, tile(blk(ha, 0), 0)),
                                blk(ha, 0)[:, LANES:]]), ha[M:]])

        keys = []
        for p in range(NP):
            ka = _dot(ha_tied if p == SIDE_TIE else ha, _unpack(ka_s[p]))
            if p == 0:
                kb = _dot(h[:, :D], _unpack(_cols([kb_s[n] for n in range(NP)])))
            keys += [_cols([ka[:, :DA], lo(tile(kb, p))]), _cols([ka[:, DA:], hi(tile(kb, p))])]

        vals = []

        def values(first, last):
            for p in range(first, last):
                v = _dot(ha, _unpack(va_s[p]))
                vals.extend([_cols([v[:, :DA], lo(v[:, 2 * DA:])]),
                             _cols([v[:, DA:2 * DA], hi(v[:, 2 * DA:])])])

        hb_rows = [_rows([lo(blk(hb, i)), hi(blk(hb, i))]) for i in range(NB)]
        hb_rows += [jnp.zeros((2 * M, LANES), F32)] * (NP - NB)
        hb_rows = [e.astype(BF16) for e in hb_rows]

        qb = _dot(ha, _unpack(_cols([qb_s[p] for p in range(NP)])))
        sb = _dot_nt(_round_bf16(_rows([tile(qb, p) for p in range(NP)])), _rows(hb_rows))
        values(0, VALUES_EARLY)
        score = {}
        for i in range(NB):
            kT_s[i] = _pack(_rows([blk(k, i) for k in keys]).T)
            t = _dot(_rows([blk(h, q) for q in seen_by[i]]), _unpack(kT_s[i]))
            for n, q in enumerate(seen_by[i]):
                score[q, i] = blk(t, n)

        prob = {}
        for q in range(NB):
            for i in sees[q]:
                t = None
                for p in range(NP):
                    r = _roll(blk(sb, p * NB + q), 2 * M * (p - i))
                    t = r if t is None else jnp.where(slot == p, r, t)
                t = score[q, i] + t
                score[q, i] = jnp.where(causal, t, -1e9) if (i == q and q > 0) else t
            mx = per_head(functools.reduce(jnp.maximum, [score[q, i] for i in sees[q]]),
                          jnp.maximum)
            ex = [jnp.exp(score[q, i] - mx) for i in sees[q]]
            inv = 1.0 / per_head(functools.reduce(jnp.add, ex), jnp.add)
            for i, e in zip(sees[q], ex):
                prob[q, i] = _round_bf16(e * inv)
        shifted = {(q, i): _roll(v, 2 * M * i) for (q, i), v in prob.items()}

        values(VALUES_EARLY, NP - VALUES_LATE)
        ub = []
        for p in range(NP):
            lhs = []
            for q in range(NB):
                t = jnp.zeros((M, LANES), F32)
                for i in sees[q]:
                    t = jnp.where(slot == (i + p) % NP, shifted[q, i], t)
                lhs.append(t)
            ub.append(_dot(_rows(lhs), _rows([hb_rows[(n - p) % NP] for n in range(NP)])))
        values(NP - VALUES_LATE, NP)
        ub = [_round_bf16(u) for u in ub]

        def expand(pairs, r0, r1):
            return _dot(_cols([ub[p][r0:r1] for p in pairs]),
                        _unpack(_rows([vb_s[p] for p in pairs])))

        fill = FILL_PAIRS if j + 1 < SPB else 0
        o = expand(range(NP - fill), 0, L)
        out = [blk(o, q) for q in range(NB)]
        if fill:
            out[0] = out[0] + expand(range(NP - fill, NP), 0, M)
        for i in range(NB):
            t = _dot(_rows([prob[q, i] for q in seen_by[i]]),
                     _rows([blk(v, i) for v in vals]).astype(BF16))
            for n, q in enumerate(seen_by[i]):
                out[q] = out[q] + blk(t, n)
        tokens = _rows(out[1:])
        if fill:
            tokens = tokens + expand(range(NP - fill, NP), M, L)
        o_s[j] = tokens
        return out[0], hn, best, bidx

    def token_block(b, carry):
        m, best, bidx = carry

        @pl.when(b == 1)
        def _():
            wait(d_mod1 + d_x1)
            for i, v in enumerate(modulation(wmod1_s)):
                mod_s[i] = v

        @pl.when(b == 2)
        def _():
            wait(d_ffn)

        hx = h_s[...]
        for j in range(SPB):
            m, hx, best, bidx = step(b, j, m, hx, best, bidx)
        h_s[...] = hx

        @pl.when(b > 0)
        def _():
            out_copy(b - 1, 1, 0).start()

        return m, best, bidx

    m0 = dup(mem0_s[...].astype(F32))
    m0 = _cols([m0[:, :DA], lo(m0[:, DA:])])
    _, best, bidx = lax.fori_loop(
        0, NBLK, token_block,
        (m0, jnp.full((8, LANES), -jnp.inf, F32), jnp.zeros((8, LANES), jnp.int32)))
    for j in range(SPB):
        best, bidx = finish(NBLK - 1, j, True, best, bidx)
    block_out(NBLK - 1)
    out_copy(NBLK - 1, 1, 0).start()

    rmax = jnp.max(best, axis=0, keepdims=True)
    idx = jnp.min(jnp.where(best == rmax, bidx, S - 1))
    hsel = jnp.broadcast_to(h2_s[pl.ds(idx, 1), :], (8, DP))[:, :D]
    g = _dot(hsel, wg_s[...])
    u = _dot(hsel, wu_s[...])
    y = _dot_nt(_round_bf16(g * jax.nn.sigmoid(g) * u), wdT_s[...])
    y = dup(y)[0:1] * jax.nn.sigmoid(rmax[:, 0:1])
    y_s[pl.ds(idx, 1), :] = y_s[pl.ds(idx, 1), :] + mod_s[3, 0:1] * y

    out_copy(0, NBLK, 0).wait()
    block_out(idx // LANES)
    fix = out_copy(idx // LANES, 1, 1)
    fix.start()
    fix.wait()


@functools.partial(jax.jit, static_argnames=("A_seg_len",))
def pallas_adaLN_cond__memory_aug_recurrent_mem_tr__moe_arch_mod__prompt_kernel(
    A_x, A_mem0, A_Wq, A_Wk, A_Wv, A_Wo, A_seg_len, B_x, B_w_r, B_w_gate, B_w_up, B_w_down,
    c, w_mod,
):
    del B_x
    _, S, D = A_x.shape
    _, H, E = A_Wq.shape
    M = A_mem0.shape[1]
    F = B_w_gate.shape[1]
    SEG = int(A_seg_len)
    DA = D // LANES * LANES
    DP = DA + LANES
    NP = H // 2
    hbm = pl.BlockSpec(memory_space=pl.ANY)
    pairs = pltpu.VMEM((NP, D, E), U32)
    outT = pl.pallas_call(
        functools.partial(_kernel, S=S, D=D, H=H, E=E, M=M, SEG=SEG),
        out_shape=jax.ShapeDtypeStruct((D, S), A_x.dtype),
        in_specs=[hbm] * 12,
        out_specs=hbm,
        scratch_shapes=[
            pltpu.VMEM((DP, S), BF16),
            pairs, pairs, pairs,
            pltpu.VMEM((NP, 2, D, E), BF16),
            pltpu.VMEM((D, F), BF16),
            pltpu.VMEM((D, F), BF16),
            pltpu.VMEM((D, F), BF16),
            pltpu.VMEM((D, 2 * D), BF16),
            pltpu.VMEM((D, 4 * D), BF16),
            pltpu.VMEM((4, 8, DP), F32),
            pltpu.VMEM((M, D), BF16),
            pltpu.VMEM((D,), BF16),
            pltpu.VMEM((1, D), BF16),
            pltpu.VMEM((NP, DA // 2, 2 * DA), U32),
            pltpu.VMEM((NP, D // 2, LANES), U32),
            pltpu.VMEM((NP, DA // 2, LANES), U32),
            pltpu.VMEM((NP, DA // 2, 2 * D), U32),
            pltpu.VMEM((NP, LANES // 2, DP), U32),
            pltpu.VMEM((S, DP), F32),
            pltpu.VMEM((SEG, DP), F32),
            pltpu.VMEM((LANES // SEG, SEG, DP), F32),
            pltpu.VMEM((S, DP), F32),
            pltpu.VMEM((S, DP), F32),
            pltpu.VMEM((DP, S), BF16),
            pltpu.VMEM(((M + SEG) // M, DP // 2, LANES), U32),
            pltpu.SemaphoreType.DMA((16 + 4 * NP,)),
            pltpu.SemaphoreType.DMA((2,)),
        ],
        compiler_params=pltpu.CompilerParams(vmem_limit_bytes=100 * 2**20),
        name="rmt_fused",
    )(
        jnp.transpose(A_x[0]),
        A_mem0[0],
        A_Wq,
        A_Wk,
        A_Wv,
        jnp.transpose(A_Wo, (0, 2, 1)),
        B_w_r,
        B_w_gate,
        B_w_up,
        jnp.transpose(B_w_down),
        c,
        w_mod,
    )
    return jnp.transpose(outT)[None]
```
